```python
import os as _os
_os.environ.setdefault("JAX_PLATFORMS", "cpu")
import jax
import jax.numpy as jnp

def _softmax(x, axis=-1):
    return jax.nn.softmax(x, axis=axis)
def _gelu(x):
    return jax.nn.gelu(x, approximate=True)
def _silu(x):
    return jax.nn.silu(x)
def _sigmoid(x):
    return jax.nn.sigmoid(x)
def _layernorm(x, axis=-1, eps=1e-5):
    m = jnp.mean(x, axis=axis, keepdims=True)
    v = jnp.var(x, axis=axis, keepdims=True)
    return (x - m) / jnp.sqrt(v + eps)
def _scatter_add(tgt, idx, src, axis=0):
    return tgt.at[idx].add(src)
def _segment_sum(src, seg, n):
    return jax.ops.segment_sum(src, seg, n)
class _Rng:
    def __init__(self, key):
        self._k = key
    def _next(self):
        self._k, sub = jax.random.split(self._k)
        return sub
    def normal(self, shape):
        return jax.random.normal(self._next(), shape, dtype=jnp.bfloat16)
    def randint(self, lo, hi, shape):
        return jax.random.randint(self._next(), shape, lo, hi, dtype=jnp.int32)
    def uniform(self, shape, lo=0.0, hi=1.0):
        return jax.random.uniform(self._next(), shape, jnp.bfloat16, lo, hi)
    def permutation(self, n):
        return jax.random.permutation(self._next(), n)


kernel_name = 'gated_mix__sliding_block_cached__swiglu_ffn__decode'

def setup_inputs():
    _rng = _Rng(jax.random.key(int.from_bytes(__import__("os").urandom(4), "little")))
    _w = (lambda a: (lambda t: t.astype(jnp.bfloat16) if jnp.issubdtype(t.dtype, jnp.floating) else t)(jnp.asarray(a)))
    def _A_setup():
        B, Sq, D = 1, 1, 512
        Hq, Hkv, Sk, Dh = 32, 32, 32768, 128
        assert Hq % Hkv == 0, (Hq, Hkv)
        return {
            "x": _w((lambda *s: _rng.normal(s) * 0.05)(B, Sq, D)),
            "k_cache": _w((lambda *s: _rng.normal(s) * 3.2)(B, Hkv, Sk, Dh)),
            "v_cache": _w((lambda *s: _rng.normal(s) * 1.6)(B, Hkv, Sk, Dh)),
            "wq": _w((lambda *s: _rng.normal(s) * 3.2)(D, Hq * Dh) * (D ** -0.5)),
            "wo": _w((lambda *s: _rng.normal(s) * 1.6)(Hq * Dh, D) * ((Hq * Dh) ** -0.5)),
        }
    _A_in = _A_setup()

    def _B_setup():
        B, S, D, F = 1, 1, 512, 1376
        return {
            "x": _w((lambda *s: _rng.normal(s) * 0.05)(B, S, D)),
            "w_gate": _w((lambda *s: _rng.normal(s) * 0.1)(D, F)),
            "w_up": _w((lambda *s: _rng.normal(s) * 0.1)(D, F)),
            "w_down": _w((lambda *s: _rng.normal(s) * 0.1)(F, D)),
        }
    _B_in = _B_setup()

    return {
        "A_x": _A_in["x"],
        "A_k_cache": _A_in["k_cache"],
        "A_v_cache": _A_in["v_cache"],
        "A_wq": _A_in["wq"],
        "A_wo": _A_in["wo"],
        "B_x": _B_in["x"],
        "B_w_gate": _B_in["w_gate"],
        "B_w_up": _B_in["w_up"],
        "B_w_down": _B_in["w_down"],
        "gate_w": _w((lambda *s: _rng.normal(s) * 0.05)(512) * 16.0),
    }

def reference(A_x, A_k_cache, A_v_cache, A_wq, A_wo, B_x, B_w_gate, B_w_up, B_w_down, gate_w):
    def _A_ref(x, k_cache, v_cache, wq, wo):
        B, Sq, D = x.shape
        Hq, Dh = 32, 128
        Hkv, Sk = k_cache.shape[1], k_cache.shape[2]
        W = min(4096, max(256, Sk // 4))
        rep = Hq // Hkv
        q = (lambda x, *d: x.transpose(*d))((x @ wq).reshape(B, Sq, Hq, Dh), 0, 2, 1, 3)
        k = jnp.repeat(k_cache[:, :, Sk - W:, :], rep, axis=1)
        v = jnp.repeat(v_cache[:, :, Sk - W:, :], rep, axis=1)
        scores = jnp.einsum("bhqd,bhkd->bhqk", q, k) * (Dh ** -0.5)
        p = _softmax(scores, axis=-1)
        o = jnp.einsum("bhqk,bhkd->bhqd", p, v)
        return (lambda x, *d: x.transpose(*d))(o, 0, 2, 1, 3).reshape(B, Sq, Hq * Dh) @ wo

    def _B_ref(x, w_gate, w_up, w_down):
        g = _silu(x @ w_gate)
        u = x @ w_up
        return (g * u) @ w_down

    x = A_x
    g = _sigmoid((x * gate_w).sum(-1, keepdims=True))
    a = _A_ref(x, A_k_cache, A_v_cache, A_wq, A_wo)
    b = _B_ref(x, B_w_gate, B_w_up, B_w_down)
    return g * a + (1 - g) * b
```

```python
import jax
import jax.numpy as jnp
from jax import lax
import jax.experimental.pallas as pl
import jax.experimental.pallas.tpu as pltpu

_F32 = jnp.float32
_NT = (((1,), (1,)), ((), ()))

_KV_ROWS = 160
_NSLOT = 3
_W_ROWS = 32
_WQ_COLS = 1024
_WO_CHUNKS = (1024, 1024, 1024, 512, 256, 128, 128)


@jax.jit
def pallas_gated_mix__sliding_block_cached__swiglu_ffn__decode_kernel(
    A_x: jax.Array,
    A_k_cache: jax.Array,
    A_v_cache: jax.Array,
    A_wq: jax.Array,
    A_wo: jax.Array,
    B_x: jax.Array,
    B_w_gate: jax.Array,
    B_w_up: jax.Array,
    B_w_down: jax.Array,
    gate_w: jax.Array,
):
    del B_x
    _, H, SK, DH = A_k_cache.shape
    D = A_x.shape[-1]
    FF = B_w_down.shape[0]
    W = min(4096, max(256, SK // 4))
    scale = DH ** -0.5
    dt = A_x.dtype
    wo_off = [sum(_WO_CHUNKS[:i]) for i in range(len(_WO_CHUNKS))]
    assert sum(_WO_CHUNKS) == H * DH

    def kern(x_hbm, k_hbm, v_hbm, wq_hbm, wo_hbm, wg_hbm, wu_hbm, wd_hbm, gw_hbm, o_ref,
             x_v, gw_v, wq_v, wo_v, ffn_v, kv_v, q_v, att_v, sem_s, sem_kv, sem_wq, sem_f, sem_wo):
        def start_kv(h, slot):
            r = 0
            while r < W:
                n = min(_KV_ROWS, W - r)
                for t in range(2):
                    src = (k_hbm, v_hbm)[t].at[0, h, pl.ds(SK - W + r, n), :]
                    pltpu.make_async_copy(src, kv_v.at[slot, t, pl.ds(r, n)], sem_kv.at[slot]).start(priority=t)
                r += n

        def wait_all(ref, sem):
            pltpu.make_async_copy(ref, ref, sem).wait()

        def wq_body(i, _):
            r = pl.multiple_of(i * 16, 16)
            for j in range(H * DH // _WQ_COLS):
                pltpu.make_async_copy(wq_hbm.at[pl.ds(r, 16), pl.ds(j * _WQ_COLS, _WQ_COLS)],
                                      wq_v.at[pl.ds(r, 16), pl.ds(j * _WQ_COLS, _WQ_COLS)], sem_wq).start(priority=j % 2)
        lax.fori_loop(0, D // 16, wq_body, None)
        cx = pltpu.make_async_copy(x_hbm, x_v, sem_s.at[0])
        cx.start()
        cg = pltpu.make_async_copy(gw_hbm, gw_v, sem_s.at[1])
        cg.start()

        def gu_body(i, _):
            r = pl.multiple_of(i * _W_ROWS, _W_ROWS)
            for t in range(2):
                pltpu.make_async_copy((wg_hbm, wu_hbm)[t].at[pl.ds(r, _W_ROWS)], ffn_v.at[t, pl.ds(r, _W_ROWS)],
                                      sem_f.at[0]).start(priority=t)
        lax.fori_loop(0, FF // _W_ROWS, gu_body, None)
        cx.wait()
        cg.wait()
        wait_all(wq_v, sem_wq)
        x = x_v[0]
        q = jnp.dot(x, wq_v[...], preferred_element_type=_F32)
        for h in range(H):
            q_v[h] = q[:, h * DH:(h + 1) * DH]

        half = FF // 2

        def dn_body(i, _):
            for t in range(2):
                r = pl.multiple_of(t * half + i * 16, 16)
                pltpu.make_async_copy(wd_hbm.at[pl.ds(r, 16)], ffn_v.at[2, pl.ds(r, 16)], sem_f.at[1]).start(priority=t)
        lax.fori_loop(0, half // 16, dn_body, None)
        wait_all(ffn_v.at[pl.ds(0, 2)], sem_f.at[0])
        g = lax.dot_general(x, ffn_v[0], _NT, preferred_element_type=_F32)
        u = lax.dot_general(x, ffn_v[1], _NT, preferred_element_type=_F32)
        hid = (g * jax.nn.sigmoid(g) * u).astype(dt)
        start_kv(0, 0)
        wait_all(ffn_v.at[2], sem_f.at[1])
        b = jnp.dot(hid, ffn_v[2], preferred_element_type=_F32)
        gate = jax.nn.sigmoid(jnp.sum(x.astype(_F32) * gw_v[...].astype(_F32).reshape(1, D), axis=-1, keepdims=True))

        def start_wo(c):
            n = _WO_CHUNKS[c] // 2

            def body(i, _):
                for t in range(2):
                    r = pl.multiple_of(wo_off[c] + t * n + i * _W_ROWS, _W_ROWS)
                    pltpu.make_async_copy(wo_hbm.at[pl.ds(r, _W_ROWS)], wo_v.at[pl.ds(r, _W_ROWS)],
                                          sem_wo.at[c]).start(priority=t)
            lax.fori_loop(0, n // _W_ROWS, body, None)

        la = _NSLOT - 1

        def pre(i, _):
            start_kv(i, i)
        lax.fori_loop(1, la, pre, None)

        def head(h, _):
            slot = h % _NSLOT

            @pl.when(h + la < H)
            def _():
                start_kv(h + la, (h + la) % _NSLOT)

            @pl.when(h + la == H)
            def _():
                start_wo(0)
                start_wo(1)

            @pl.when(h + la == H + 1)
            def _():
                for c in range(2, len(_WO_CHUNKS)):
                    start_wo(c)
            wait_all(kv_v.at[slot], sem_kv.at[slot])
            s = lax.dot_general(q_v[h].astype(dt), kv_v[slot, 0], _NT, preferred_element_type=_F32) * scale
            m = jnp.max(s, axis=-1, keepdims=True)
            p = jnp.exp(s - m)
            l = jnp.sum(p, axis=-1, keepdims=True)
            o = jnp.dot(p.astype(dt), kv_v[slot, 1], preferred_element_type=_F32)
            att_v[h] = o / l
        lax.fori_loop(0, H, head, None)

        a = jnp.zeros((1, D), _F32)
        for c in range(len(_WO_CHUNKS)):
            wait_all(wo_v.at[pl.ds(wo_off[c], _WO_CHUNKS[c])], sem_wo.at[c])
            h0 = wo_off[c] // DH
            oc = jnp.concatenate([att_v[h0 + j] for j in range(_WO_CHUNKS[c] // DH)], axis=-1).astype(dt)
            a = a + jnp.dot(oc, wo_v[pl.ds(wo_off[c], _WO_CHUNKS[c]), :], preferred_element_type=_F32)
        o_ref[0] = (gate * a + (1.0 - gate) * b).astype(o_ref.dtype)

    hbm = pl.BlockSpec(memory_space=pltpu.HBM)
    return pl.pallas_call(
        kern,
        out_shape=jax.ShapeDtypeStruct(A_x.shape, dt),
        in_specs=[hbm] * 9,
        scratch_shapes=[
            pltpu.VMEM(A_x.shape, dt), pltpu.VMEM(gate_w.shape, dt),
            pltpu.VMEM(A_wq.shape, dt), pltpu.VMEM(A_wo.shape, dt),
            pltpu.VMEM((3, FF, D), dt), pltpu.VMEM((_NSLOT, 2, W, DH), dt),
            pltpu.VMEM((H, 1, DH), _F32), pltpu.VMEM((H, 1, DH), _F32),
            pltpu.SemaphoreType.DMA((2,)), pltpu.SemaphoreType.DMA((_NSLOT,)), pltpu.SemaphoreType.DMA(()),
            pltpu.SemaphoreType.DMA((2,)), pltpu.SemaphoreType.DMA((len(_WO_CHUNKS),)),
        ],
        compiler_params=pltpu.CompilerParams(vmem_limit_bytes=64 * 2**20),
    )(A_x, A_k_cache, A_v_cache, A_wq, A_wo, B_w_gate.T, B_w_up.T, B_w_down, gate_w)
```

```python
import functools

import jax
import jax.numpy as jnp
from jax import lax
import jax.experimental.pallas as pl
import jax.experimental.pallas.tpu as pltpu

_F32 = jnp.float32
_NT = (((1,), (1,)), ((), ()))

_GROUP = 8
_LAG = _GROUP + 1
_KV_ROWS = 64
_STREAMS = 8
_W_ROWS = 32
_WQ_ROWS, _WQ_COLS = 8, 1024
_LAST = 2


def _window(sk):
    return min(4096, max(256, sk // 4))


def _start(src, dst, sem, priority):
    pltpu.make_async_copy(src, dst, sem).start(priority=priority)


def _wait_filled(ref, sem):
    pltpu.make_async_copy(ref, ref, sem).wait()


def _body(x_hbm, k_hbm, v_hbm, wq_hbm, wo_hbm, wg_hbm, wu_hbm, wd_hbm, gw_hbm,
          o_ref,
          x_v, gw_v, wq_v, wo_v, ffn_v, kv_v, q_v, att_v, col_v,
          sem_x, sem_gw, sem_wq, sem_kv, sem_ffn, sem_wo):
    _, H, SK, DH = k_hbm.shape
    D = x_v.shape[-1]
    FF = ffn_v.shape[1]
    W = _window(SK)
    HS = H // _STREAMS
    dtype = x_v.dtype

    def wq_round(i, _, *, alternate):
        per_row = H * DH // (2 * _WQ_COLS)
        for j in range(_STREAMS):
            r = pl.multiple_of(j * (D // _STREAMS) + (i // per_row) * _WQ_ROWS, _WQ_ROWS)
            for z in range(2):
                c = pl.multiple_of((2 * (i % per_row) + z) * _WQ_COLS, _WQ_COLS)
                ix = (pl.ds(r, _WQ_ROWS), pl.ds(c, _WQ_COLS))
                _start(wq_hbm.at[ix], wq_v.at[ix], sem_wq, j % 2 if alternate else 1)

    def kv_round(i, _):
        g = i // (W // _KV_ROWS)
        r = pl.multiple_of((i % (W // _KV_ROWS)) * _KV_ROWS, _KV_ROWS)
        for j in range(0, _GROUP, 2):
            for t, src in enumerate((k_hbm, v_hbm)):
                _start(src.at[0, pl.ds(g * _GROUP + j, 2), pl.ds(SK - W + r, _KV_ROWS)],
                       kv_v.at[g, t, pl.ds(j, 2), pl.ds(r, _KV_ROWS)], sem_kv.at[g], t)

    def ffn_rows(r, parity):
        for t, src in enumerate((wg_hbm, wu_hbm, wd_hbm)):
            _start(src.at[pl.ds(r, _W_ROWS)], ffn_v.at[t, pl.ds(r, _W_ROWS)], sem_ffn,
                   (parity + t) % 2)

    n_ffn = FF // _W_ROWS // 2

    def ffn_round(i, _):
        ffn_rows(pl.multiple_of(i * _W_ROWS, _W_ROWS), 0)
        ffn_rows(pl.multiple_of((n_ffn + i) * _W_ROWS, _W_ROWS), 1)

    def wo_rows(c, s, r, sem, priority):
        r0 = (s * HS + c) * DH + r
        if not isinstance(r0, int):
            r0 = pl.multiple_of(r0, _W_ROWS)
        _start(wo_hbm.at[pl.ds(r0, _W_ROWS)], wo_v.at[c, s, pl.ds(r, _W_ROWS)], sem, priority)

    def wo_half_round(i, _):
        c = i // (2 * DH // _W_ROWS)
        r = pl.multiple_of((i // 2) % (DH // _W_ROWS) * _W_ROWS, _W_ROWS)
        for j in range(_STREAMS // 2):
            wo_rows(c, (i % 2) * (_STREAMS // 2) + j, r, sem_wo.at[c], j % 2)

    n_wq = D // _STREAMS // _WQ_ROWS * (H * DH // (2 * _WQ_COLS))
    n_wo = (HS - 1) * 2 * DH // _W_ROWS

    def kv_issued(s):
        return jnp.minimum(s + 1, H) * (W // _KV_ROWS // _GROUP)

    def ffn_issued(s):
        return jnp.where(s < H, 0, jnp.where(s == H, 10, jnp.minimum(12 + 3 * (s - H), n_ffn)))

    def wo_issued(s):
        return jnp.clip(5 * (s - H - 3), 0, n_wo)

    assert 10 <= n_ffn <= 12 + 3 * (_LAG - 1) and n_wo <= 5 * (_LAG - 4)

    lax.fori_loop(0, 2, functools.partial(wq_round, alternate=False), None)
    lax.fori_loop(2, n_wq, functools.partial(wq_round, alternate=True), None)
    _start(x_hbm, x_v, sem_x, 0)
    _start(gw_hbm, gw_v, sem_gw, 0)

    def step(s, _):
        lax.fori_loop(kv_issued(s - 1), kv_issued(s), kv_round, None)
        if FF // _W_ROWS % 2:
            pl.when(s == H)(lambda: ffn_rows(FF - _W_ROWS, 1))
        lax.fori_loop(ffn_issued(s - 1), ffn_issued(s), ffn_round, None)
        lax.fori_loop(wo_issued(s - 1), wo_issued(s), wo_half_round, None)

        @pl.when(s == 1)
        def _():
            _wait_filled(x_v, sem_x)
            _wait_filled(wq_v, sem_wq)
            q = jnp.dot(x_v[0], wq_v[...], preferred_element_type=_F32)
            for h in range(H):
                q_v[h] = q[:, h * DH:(h + 1) * DH]

        @pl.when(s >= _LAG)
        def _():
            h = s - _LAG
            g, j = h // _GROUP, h % _GROUP
            pl.when(j == 0)(lambda: _wait_filled(kv_v.at[g], sem_kv.at[g]))
            scores = lax.dot_general(q_v[h].astype(dtype), kv_v[g, 0, j], _NT,
                                     preferred_element_type=_F32) * DH ** -0.5
            p = jnp.exp(scores - jnp.max(scores, axis=-1, keepdims=True))
            o = jnp.dot(p.astype(dtype), kv_v[g, 1, j], preferred_element_type=_F32)
            att_v[h] = o / jnp.sum(p, axis=-1, keepdims=True)

    lax.fori_loop(0, H + _LAG, step, None)

    x = x_v[0]
    _wait_filled(gw_v, sem_gw)
    _wait_filled(ffn_v, sem_ffn)
    gate = jax.nn.sigmoid(jnp.sum(
        x.astype(_F32) * gw_v[...].astype(_F32).reshape(1, D), axis=-1, keepdims=True))
    up_g = lax.dot_general(x, ffn_v[0], _NT, preferred_element_type=_F32)
    up_u = lax.dot_general(x, ffn_v[1], _NT, preferred_element_type=_F32)
    hidden = (up_g * jax.nn.sigmoid(up_g) * up_u).astype(dtype)

    n_mxu = _STREAMS - _LAST
    for r in range(0, DH, _W_ROWS):
        for s in range(n_mxu):
            wo_rows(HS - 1, s, r, sem_wo.at[HS - 1], s % 2)
    for r in range(0, DH, _W_ROWS):
        for s in range(n_mxu, _STREAMS):
            wo_rows(HS - 1, s, r, sem_wo.at[HS], 1)

    out = (1.0 - gate) * jnp.dot(hidden, ffn_v[2], preferred_element_type=_F32)

    def project(c, n):
        return gate * functools.reduce(jnp.add, [
            jnp.dot(att_v[s * HS + c].astype(dtype), wo_v[c, s], preferred_element_type=_F32)
            for s in range(n)])

    def wo_chunk(c, out):
        _wait_filled(wo_v.at[c], sem_wo.at[c])
        return out + project(c, _STREAMS)

    for i in range(_LAST):
        o = gate * att_v[(n_mxu + i) * HS + HS - 1]
        col_v[i] = jnp.broadcast_to(o, (DH, DH)).T
    out = lax.fori_loop(0, HS - 1, wo_chunk, out)
    _wait_filled(wo_v.at[HS - 1, pl.ds(0, n_mxu)], sem_wo.at[HS - 1])
    out = out + project(HS - 1, n_mxu)
    _wait_filled(wo_v.at[HS - 1, pl.ds(n_mxu, _LAST)], sem_wo.at[HS])
    out = out + jnp.concatenate([
        jnp.sum(functools.reduce(jnp.add, [
            col_v[i] * wo_v[HS - 1, n_mxu + i, :, pl.ds(c, DH)].astype(_F32)
            for i in range(_LAST)]), axis=0, keepdims=True)
        for c in range(0, D, DH)], axis=1)
    o_ref[0] = out.astype(o_ref.dtype)


@jax.jit
def pallas_gated_mix__sliding_block_cached__swiglu_ffn__decode_kernel(
    A_x: jax.Array,
    A_k_cache: jax.Array,
    A_v_cache: jax.Array,
    A_wq: jax.Array,
    A_wo: jax.Array,
    B_x: jax.Array,
    B_w_gate: jax.Array,
    B_w_up: jax.Array,
    B_w_down: jax.Array,
    gate_w: jax.Array,
):
    del B_x
    _, H, SK, DH = A_k_cache.shape
    D = A_x.shape[-1]
    FF = B_w_down.shape[0]
    W = _window(SK)
    dtype = A_x.dtype
    assert A_x.shape == (1, 1, D) and A_wq.shape == (D, H * DH) and A_wo.shape == (H * DH, D)
    assert H % _GROUP == 0 and H % _STREAMS == 0 and W % (_KV_ROWS * _GROUP) == 0
    assert FF % _W_ROWS == 0 and DH % _W_ROWS == 0 and D % DH == 0
    assert D % (_STREAMS * _WQ_ROWS) == 0 and H * DH % (2 * _WQ_COLS) == 0

    def kernel(*refs):
        dma = pltpu.SemaphoreType.DMA
        pl.run_scoped(functools.partial(_body, *refs),
                      dma(()), dma(()), dma(()), dma((H // _GROUP,)), dma(()),
                      dma((H // _STREAMS + 1,)))

    return pl.pallas_call(
        kernel,
        out_shape=jax.ShapeDtypeStruct(A_x.shape, dtype),
        in_specs=[pl.BlockSpec(memory_space=pltpu.HBM)] * 9,
        scratch_shapes=[
            pltpu.VMEM(A_x.shape, dtype),
            pltpu.VMEM(gate_w.shape, dtype),
            pltpu.VMEM(A_wq.shape, dtype),
            pltpu.VMEM((H // _STREAMS, _STREAMS, DH, D), dtype),
            pltpu.VMEM((3, FF, D), dtype),
            pltpu.VMEM((H // _GROUP, 2, _GROUP, W, DH), dtype),
            pltpu.VMEM((H, 1, DH), _F32),
            pltpu.VMEM((H, 1, DH), _F32),
            pltpu.VMEM((_LAST, DH, DH), _F32),
        ],
        compiler_params=pltpu.CompilerParams(
            vmem_limit_bytes=100 * 2**20,
            disable_bounds_checks=True,
        ),
    )(A_x, A_k_cache, A_v_cache, A_wq, A_wo, B_w_gate.T, B_w_up.T, B_w_down, gate_w)
```
